```python
import os as _os
_os.environ.setdefault('JAX_PLATFORMS', 'cpu')
import jax
import jax.numpy as jnp

def _softmax(x, axis=-1):
    return jax.nn.softmax(x, axis=axis)

def _gelu(x):
    return jax.nn.gelu(x, approximate=True)

def _silu(x):
    return jax.nn.silu(x)

def _sigmoid(x):
    return jax.nn.sigmoid(x)

def _layernorm(x, axis=-1, eps=1e-05):
    m = jnp.mean(x, axis=axis, keepdims=True)
    v = jnp.var(x, axis=axis, keepdims=True)
    return (x - m) / jnp.sqrt(v + eps)

def _scatter_add(tgt, idx, src, axis=0):
    return tgt.at[idx].add(src)

def _segment_sum(src, seg, n):
    return jax.ops.segment_sum(src, seg, n)

class _Rng:

    def __init__(self, key):
        self._k = key

    def _next(self):
        self._k, sub = jax.random.split(self._k)
        return sub

    def normal(self, shape):
        return jax.random.normal(self._next(), shape, dtype=jnp.bfloat16)

    def randint(self, lo, hi, shape):
        return jax.random.randint(self._next(), shape, lo, hi, dtype=jnp.int32)

    def uniform(self, shape, lo=0.0, hi=1.0):
        return jax.random.uniform(self._next(), shape, jnp.bfloat16, lo, hi)

    def permutation(self, n):
        return jax.random.permutation(self._next(), n)
kernel_name = 'adaLN_cond__sliding_local_dilated__dense_activation_relu__prompt'

def setup_inputs():
    _rng = _Rng(jax.random.key(int.from_bytes(__import__("os").urandom(4), "little")))
    _w = lambda a: (lambda t: t.astype(jnp.bfloat16) if jnp.issubdtype(t.dtype, jnp.floating) else t)(jnp.asarray(a))

    def _A_setup():
        B, S, D = (1, 2048, 576)
        return {'x': _w((lambda *s: _rng.normal(s) * 0.05)(B, S, D)), 'wqkv': _w((lambda *s: _rng.normal(s) * 0.05)(D, 3 * D)), 'wo': _w((lambda *s: _rng.normal(s) * 0.05)(D, D))}
    _A_in = _A_setup()

    def _B_setup():
        B, S, D, Dff = (1, 2048, 576, 4608)
        return {'x': _w((lambda *s: _rng.normal(s) * 0.05)(B, S, D)), 'w1': _w((lambda *s: _rng.normal(s) * 0.05)(D, Dff)), 'w2': _w((lambda *s: _rng.normal(s) * 0.05)(Dff, D))}
    _B_in = _B_setup()
    return {'A_x': _A_in['x'], 'A_wqkv': _A_in['wqkv'], 'A_wo': _A_in['wo'], 'B_x': _B_in['x'], 'B_w1': _B_in['w1'], 'B_w2': _B_in['w2'], 'c': _w((lambda *s: _rng.normal(s) * 0.05)(1, 576) * 8.0), 'w_mod': _w((lambda *s: _rng.normal(s) * 0.05)(576, 6 * 576) * 576 ** (-0.5) * 8.0)}

def reference(A_x, A_wqkv, A_wo, B_x, B_w1, B_w2, c, w_mod):

    def _A_ref(x, wqkv, wo):
        B, S, D = x.shape
        H = 32
        Dh = D // H
        W, dil = (8, 2)
        qkv = (lambda x, *d: x.transpose(*d))((x @ wqkv).reshape(B, S, 3, H, Dh), 2, 0, 3, 1, 4)
        q, k, v = (qkv[0], qkv[1], qkv[2])
        scale = Dh ** (-0.5)
        pos = jnp.arange(S)
        off = jnp.arange(W) * dil
        idx = pos[:, None] - off[None, :]
        mask = idx >= 0
        idx_c = jnp.where(mask, idx, 0).reshape(-1)
        kg = k[:, :, idx_c, :].reshape(B, H, S, W, Dh)
        vg = v[:, :, idx_c, :].reshape(B, H, S, W, Dh)
        logits = jnp.einsum('bhsd,bhswd->bhsw', q, kg) * scale
        logits = jnp.where(mask[None, None, :, :], logits, -1000000000.0)
        attn = _softmax(logits, axis=-1)
        o = jnp.einsum('bhsw,bhswd->bhsd', attn, vg)
        return (lambda x, *d: x.transpose(*d))(o, 0, 2, 1, 3).reshape(B, S, D) @ wo

    def _B_ref(x, w1, w2):
        h = jnp.einsum('bsd,df->bsf', x, w1)
        zero = jnp.zeros_like(h)
        h = jnp.maximum(h, zero)
        return jnp.einsum('bsf,fd->bsd', h, w2)
    x = A_x
    mod = (_silu(c) @ w_mod).reshape(c.shape[0], 6, 1, -1)
    sa, ca, ga, sb, cb, gb = (mod[:, 0].copy(), mod[:, 1].copy(), mod[:, 2].copy(), mod[:, 3].copy(), mod[:, 4].copy(), mod[:, 5].copy())
    h = _layernorm(x, axis=-1) * (1 + ca) + sa
    x = x + ga * _A_ref(h, A_wqkv, A_wo)
    h = _layernorm(x, axis=-1) * (1 + cb) + sb
    x = x + gb * _B_ref(h, B_w1, B_w2)
    return x
```

```python
import functools

import jax
import jax.numpy as jnp
import jax.experimental.pallas as pl
import jax.experimental.pallas.tpu as pltpu

S = 2048
D = 576
H = 32
DH = 18
W = 8
DIL = 2
DFF = 4608
HALO = 128
T = 512
FC = 512
EPS = 1e-5


def _ln0(x):
    m = jnp.mean(x, axis=0, keepdims=True)
    xc = x - m
    v = jnp.mean(xc * xc, axis=0, keepdims=True)
    return xc * jax.lax.rsqrt(v + EPS)


def _rep(col):
    return jnp.concatenate([col] * (T // 128), axis=1)


def _kernel(x_ref, c_hbm, wmod_hbm, wqkv_hbm, wo_hbm, w1_hbm, w2t_hbm, o_ref,
            c_v, wmod_v, wqkv_v, wo_v, w1_v, w2t_v,
            mod_s, tmp_s, wqkvt_s, wot_s, w1t_s, k_s, v_s, sems):
    step = pl.program_id(0)

    srcs = (c_hbm, wmod_hbm, wqkv_hbm, wo_hbm, w1_hbm, w2t_hbm)
    dsts = (c_v, wmod_v, wqkv_v, wo_v, w1_v, w2t_v)
    copies = [pltpu.make_async_copy(s, d, sems.at[i])
              for i, (s, d) in enumerate(zip(srcs, dsts))]

    def put_tmp(a):
        for j in range(5):
            wdt = min(128, D - j * 128)
            tmp_s[j, :, 0:wdt] = a[:, j * 128:j * 128 + wdt]

    def get_rows(d):
        blks = []
        for j in range(5):
            wdt = min(128, D - j * 128)
            blks.append(tmp_s[j, pl.ds(d, H, stride=DH), :][:, 0:wdt])
        return jnp.concatenate(blks, axis=1)

    @pl.when(step == 0)
    def _():
        for cp in copies:
            cp.start()
        k_s[:, 0:HALO] = jnp.zeros((D, HALO), jnp.float32)
        v_s[:, 0:HALO] = jnp.zeros((D, HALO), jnp.float32)

        copies[0].wait()
        copies[1].wait()
        c = c_v[...].astype(jnp.float32)
        sc = c * jax.nn.sigmoid(c)
        sc_col = jnp.broadcast_to(sc, (128, D)).T
        parts = []
        for j in range(6 * D // 128):
            blk = wmod_v[:, j * 128:(j + 1) * 128].astype(jnp.float32)
            parts.append(jnp.sum(blk * sc_col, axis=0, keepdims=True))
        mod_row = jnp.concatenate(parts, axis=1)
        mod_s[...] = jnp.broadcast_to(mod_row, (128, 6 * D)).T

        copies[2].wait()
        for sec in range(3):
            put_tmp(wqkv_v[:, sec * D:(sec + 1) * D].astype(jnp.float32).T)
            for d in range(DH):
                wqkvt_s[sec * D + d * H:sec * D + (d + 1) * H, :] = (
                    get_rows(d).astype(jnp.bfloat16))
        copies[3].wait()
        put_tmp(wo_v[...].astype(jnp.float32))
        rows = [get_rows(d) for d in range(DH)]
        wot_s[...] = jnp.concatenate(rows, axis=0).T.astype(jnp.bfloat16)
        copies[4].wait()
        for j in range(DFF // 512):
            w1t_s[j * 512:(j + 1) * 512, :] = w1_v[:, j * 512:(j + 1) * 512].T
        copies[5].wait()

    def modc(i):
        return _rep(mod_s[i * D:(i + 1) * D, :])

    x = x_ref[0].astype(jnp.float32)
    h = (_ln0(x) * (1.0 + modc(1)) + modc(0)).astype(jnp.bfloat16)
    qkv = jnp.dot(wqkvt_s[...], h, preferred_element_type=jnp.float32)
    q = qkv[0:D] * (DH ** -0.5)
    k_s[:, HALO:HALO + T] = qkv[D:2 * D]
    v_s[:, HALO:HALO + T] = qkv[2 * D:3 * D]

    pos = step * T + jax.lax.broadcasted_iota(jnp.int32, (H, T), 1)
    logits = []
    for w in range(W):
        p = q * k_s[:, HALO - DIL * w:HALO - DIL * w + T]
        r = p[0:H]
        for d in range(1, DH):
            r = r + p[d * H:(d + 1) * H]
        logits.append(jnp.where(pos >= DIL * w, r, -1e9))
    m = functools.reduce(jnp.maximum, logits)
    es = [jnp.exp(l - m) for l in logits]
    inv = 1.0 / functools.reduce(lambda a, b: a + b, es)
    o = None
    for w in range(W):
        a = es[w] * inv
        t = jnp.concatenate([a] * DH, axis=0) * v_s[:, HALO - DIL * w:HALO - DIL * w + T]
        o = t if o is None else o + t
    k_s[:, 0:HALO] = k_s[:, T:T + HALO]
    v_s[:, 0:HALO] = v_s[:, T:T + HALO]

    att = jnp.dot(wot_s[...], o.astype(jnp.bfloat16), preferred_element_type=jnp.float32)
    x1 = x + modc(2) * att
    h2 = (_ln0(x1) * (1.0 + modc(4)) + modc(3)).astype(jnp.bfloat16)
    acc = None
    for f in range(DFF // FC):
        h1 = jnp.dot(w1t_s[f * FC:(f + 1) * FC, :], h2, preferred_element_type=jnp.float32)
        h1 = jnp.maximum(h1, 0.0).astype(jnp.bfloat16)
        part = jnp.dot(w2t_v[:, f * FC:(f + 1) * FC], h1, preferred_element_type=jnp.float32)
        acc = part if acc is None else acc + part
    o_ref[0] = (x1 + modc(5) * acc).astype(o_ref.dtype)


@jax.jit
def pallas_adaLN_cond__sliding_local_dilated__dense_activation_relu__prompt_kernel(
    A_x: jax.Array,
    A_wqkv: jax.Array,
    A_wo: jax.Array,
    B_x: jax.Array,
    B_w1: jax.Array,
    B_w2: jax.Array,
    c: jax.Array,
    w_mod: jax.Array,
):
    del B_x
    xt = jnp.swapaxes(A_x, 1, 2)
    w2t = B_w2.T
    hbm = pl.BlockSpec(memory_space=pl.ANY)
    out_t = pl.pallas_call(
        _kernel,
        grid=(S // T,),
        in_specs=[pl.BlockSpec((1, D, T), lambda i: (0, 0, i)),
                  hbm, hbm, hbm, hbm, hbm, hbm],
        out_specs=pl.BlockSpec((1, D, T), lambda i: (0, 0, i)),
        out_shape=jax.ShapeDtypeStruct(xt.shape, xt.dtype),
        scratch_shapes=[
            pltpu.VMEM((1, D), jnp.bfloat16),
            pltpu.VMEM((D, 6 * D), jnp.bfloat16),
            pltpu.VMEM((D, 3 * D), jnp.bfloat16),
            pltpu.VMEM((D, D), jnp.bfloat16),
            pltpu.VMEM((D, DFF), jnp.bfloat16),
            pltpu.VMEM((D, DFF), jnp.bfloat16),
            pltpu.VMEM((6 * D, 128), jnp.float32),
            pltpu.VMEM((5, D, 128), jnp.float32),
            pltpu.VMEM((3 * D, D), jnp.bfloat16),
            pltpu.VMEM((D, D), jnp.bfloat16),
            pltpu.VMEM((DFF, D), jnp.bfloat16),
            pltpu.VMEM((D, HALO + T), jnp.float32),
            pltpu.VMEM((D, HALO + T), jnp.float32),
            pltpu.SemaphoreType.DMA((6,)),
        ],
        compiler_params=pltpu.CompilerParams(
            dimension_semantics=("arbitrary",),
            vmem_limit_bytes=100 * 1024 * 1024,
        ),
    )(xt, c, w_mod, A_wqkv, A_wo, B_w1, w2t)
    return jnp.swapaxes(out_t, 1, 2)
```

```python
import functools

import jax
import jax.numpy as jnp
import jax.experimental.pallas as pl
import jax.experimental.pallas.tpu as pltpu

S = 2048
D = 576
H = 32
DH = 18
W = 8
DIL = 2
DFF = 4608
NB = 16
L = S // NB
G = 4
T = G * L
FC = 512
EPS = 1e-5
NCB = 5


def _ln0(x):
    m = jnp.mean(x, axis=0, keepdims=True)
    xc = x - m
    v = jnp.mean(xc * xc, axis=0, keepdims=True)
    return xc * jax.lax.rsqrt(v + EPS)


def _cbw(j):
    return min(128, D - j * 128)


def _kernel(x_hbm, c_hbm, wmod_hbm, wqkv_hbm, wo_hbm, w1_hbm, w2t_hbm, o_hbm,
            x_v, y_v, h_s, c_v, wmod_v, wqkv_v, wo_v, w1_v, w2t_v,
            mod_s, tmp_s, wqkvt_s, wot_s, w1t_s, nat_s, xp_s,
            q_s, k_s, v_s, ksh_s, vsh_s, o_s, sems):

    def cp(i, src, dst):
        return pltpu.make_async_copy(src, dst, sems.at[i])

    MA = 2 * D
    cp_c = cp(0, c_hbm, c_v)
    cp_ma = cp(1, wmod_hbm.at[:, 0:MA], wmod_v.at[:, 0:MA])
    QS = 512
    cp_kv = cp(2, wqkv_hbm.at[:, QS:3 * D], wqkv_v.at[:, QS:3 * D])
    cp_q = cp(7, wqkv_hbm.at[:, 0:QS], wqkv_v.at[:, 0:QS])
    cp_mb = cp(3, wmod_hbm.at[:, MA:6 * D], wmod_v.at[:, MA:6 * D])
    cp_wo = cp(4, wo_hbm, wo_v)
    cp_w1 = cp(5, w1_hbm, w1_v)
    cp_w2 = cp(6, w2t_hbm, w2t_v)

    def put_tmp(a):
        for j in range(NCB):
            tmp_s[j, :, 0:_cbw(j)] = a[:, j * 128:j * 128 + _cbw(j)]

    def get_rows(d):
        return jnp.concatenate(
            [tmp_s[j, pl.ds(d, H, stride=DH), :][:, 0:_cbw(j)] for j in range(NCB)],
            axis=1)

    def mod_cols(lo, hi):
        c = c_v[...].astype(jnp.float32)
        sc = c * jax.nn.sigmoid(c)
        sc_col = jnp.broadcast_to(sc, (128, D)).T
        parts = []
        for j in range(lo // 128, hi // 128):
            blk = wmod_v[:, j * 128:(j + 1) * 128].astype(jnp.float32)
            parts.append(jnp.sum(blk * sc_col, axis=0, keepdims=True))
        mod_row = jnp.concatenate(parts, axis=1)
        mod_s[lo:hi, :] = jnp.broadcast_to(mod_row, (128, hi - lo)).T

    def modc(i):
        col = mod_s[i * D:(i + 1) * D, :]
        return jnp.concatenate([col] * G, axis=1)

    NG = NB // G
    NF = DFF // FC
    NR = S // 512
    cp_xs = [cp(8 + r, x_hbm.at[0, :, r * 512:(r + 1) * 512],
                x_v.at[:, r * 512:(r + 1) * 512]) for r in range(NR)]
    cp_os = [cp(8 + NR + r, y_v.at[:, r * 512:(r + 1) * 512],
                o_hbm.at[0, :, r * 512:(r + 1) * 512]) for r in range(NR)]
    for c_ in cp_xs:
        c_.start()
    PW = _cbw(NCB - 1)
    tmp_s[NCB - 1, :, PW:128] = jnp.zeros((D, 128 - PW), jnp.float32)
    nat_s[NCB - 1, :, PW:128] = jnp.zeros((S, 128 - PW), jnp.float32)

    for r in range(NR):
        cp_xs[r].wait()
        if r == 0:
            cp_c.start()
            cp_ma.start()
            cp_kv.start()
        xn = x_v[:, r * 512:(r + 1) * 512].astype(jnp.float32).T
        for j in range(NCB):
            nat_s[j, r * 512:(r + 1) * 512, 0:_cbw(j)] = xn[:, j * 128:j * 128 + _cbw(j)]

    def prep_qkv(sec):
        put_tmp(wqkv_v[:, sec * D:(sec + 1) * D].astype(jnp.float32).T)
        for d in range(DH):
            wqkvt_s[sec * D + d * H:sec * D + (d + 1) * H, :] = (
                get_rows(d).astype(jnp.bfloat16))

    def gather(g):
        for i in range(G):
            b = g * G + i
            rows = jnp.concatenate(
                [nat_s[j, pl.ds(b, L, stride=NB), :][:, 0:_cbw(j)] for j in range(NCB)],
                axis=1)
            xp_s[:, b * L:(b + 1) * L] = rows.T

    def ln1(g):
        x = xp_s[:, g * T:(g + 1) * T]
        h_s[:, g * T:(g + 1) * T] = (
            _ln0(x) * (1.0 + modc(1)) + modc(0)).astype(jnp.bfloat16)

    def kvproj(g):
        kv = jnp.dot(wqkvt_s[D:3 * D, :], h_s[:, g * T:(g + 1) * T],
                     preferred_element_type=jnp.float32)
        for i in range(G):
            b = g * G + i
            kb = kv[0:D, i * L:(i + 1) * L]
            vb = kv[D:2 * D, i * L:(i + 1) * L]
            k_s[b] = kb
            v_s[b] = vb
            if b >= DIL:
                ksh_s[b] = pltpu.roll(kb, 1, 1)
                vsh_s[b] = pltpu.roll(vb, 1, 1)

    gather(0)
    cp_c.wait()
    cp_ma.wait()
    cp_q.start()
    cp_mb.start()
    cp_wo.start()
    mod_cols(0, MA)
    ln1(0)
    cp_kv.wait()
    cp_w1.start()
    prep_qkv(1)
    prep_qkv(2)

    kvproj(0)
    for g in range(1, NG):
        gather(g)
        ln1(g)
    kvproj(1)
    cp_q.wait()
    cp_mb.wait()
    cp_wo.wait()
    cp_w2.start()
    kvproj(2)
    prep_qkv(0)
    mod_cols(MA, 6 * D)
    put_tmp(wo_v[...].astype(jnp.float32))
    wot_s[...] = jnp.concatenate([get_rows(d) for d in range(DH)],
                                 axis=0).T.astype(jnp.bfloat16)
    kvproj(3)
    cp_w1.wait()

    lane0 = jax.lax.broadcasted_iota(jnp.int32, (H, L), 1) == 0

    def qproj(g):
        q = jnp.dot(wqkvt_s[0:D, :], h_s[:, g * T:(g + 1) * T],
                    preferred_element_type=jnp.float32)
        for i in range(G):
            q_s[g * G + i] = q[:, i * L:(i + 1) * L] * (DH ** -0.5)

    def attention(b):
        def src(plain, shifted, w):
            bb = b - DIL * w
            return plain.at[bb] if bb >= 0 else shifted.at[bb + NB]

        logits = [None] * W
        for d in range(DH):
            qd = q_s[b, d * H:(d + 1) * H, :]
            for w in range(W):
                t = qd * src(k_s, ksh_s, w)[d * H:(d + 1) * H, :]
                logits[w] = t if logits[w] is None else logits[w] + t
        logits = [l if b - DIL * w >= 0 else jnp.where(lane0, -1e9, l)
                  for w, l in enumerate(logits)]
        m = functools.reduce(jnp.maximum, logits)
        es = [jnp.exp(l - m) for l in logits]
        inv = 1.0 / functools.reduce(lambda a, c: a + c, es)
        ps = [e * inv for e in es]
        for d in range(DH):
            o = None
            for w in range(W):
                t = ps[w] * src(v_s, vsh_s, w)[d * H:(d + 1) * H, :]
                o = t if o is None else o + t
            o_s[d * H:(d + 1) * H, b * L:(b + 1) * L] = o.astype(jnp.bfloat16)

    def put_out(g, y):
        for i in range(G):
            b = g * G + i
            rows = y[:, i * L:(i + 1) * L].T
            for j in range(NCB):
                nat_s[j, pl.ds(b, L, stride=NB), 0:_cbw(j)] = rows[:, j * 128:j * 128 + _cbw(j)]

    def mix(g):
        att = jnp.dot(wot_s[...], o_s[:, g * T:(g + 1) * T],
                      preferred_element_type=jnp.float32)
        put_out(g, xp_s[:, g * T:(g + 1) * T] + modc(2) * att)

    def natural(r):
        x1 = jnp.concatenate(
            [nat_s[j, r * T:(r + 1) * T, 0:_cbw(j)] for j in range(NCB)], axis=1).T
        h2 = (_ln0(x1) * (1.0 + modc(4)) + modc(3)).astype(jnp.bfloat16)
        return x1, h2

    def attention_group(g):
        for i in range(G):
            attention(g * G + i)

    qproj(0)
    for j in range(DFF // 512):
        w1t_s[j * 512:(j + 1) * 512, :] = w1_v[:, j * 512:(j + 1) * 512].T
    for g in range(1, NG):
        qproj(g)
        attention_group(g - 1)
    mix(0)
    attention_group(NG - 1)
    for g in range(1, NG):
        mix(g)
    cp_w2.wait()

    nxt = natural(0)
    for r in range(NR):
        x1, h2 = nxt
        acc = None
        for f in range(NF):
            h1 = jnp.dot(w1t_s[f * FC:(f + 1) * FC, :], h2,
                         preferred_element_type=jnp.float32)
            h1 = jnp.maximum(h1, 0.0).astype(jnp.bfloat16)
            part = jnp.dot(w2t_v[:, f * FC:(f + 1) * FC], h1,
                           preferred_element_type=jnp.float32)
            acc = part if acc is None else acc + part
            if r + 1 < NR and f == NF - 3:
                nxt = natural(r + 1)
        y_v[:, r * T:(r + 1) * T] = (x1 + modc(5) * acc).astype(y_v.dtype)
        cp_os[r].start()
    for r in range(NR):
        cp_os[r].wait()


@jax.jit
def pallas_adaLN_cond__sliding_local_dilated__dense_activation_relu__prompt_kernel(
    A_x: jax.Array,
    A_wqkv: jax.Array,
    A_wo: jax.Array,
    B_x: jax.Array,
    B_w1: jax.Array,
    B_w2: jax.Array,
    c: jax.Array,
    w_mod: jax.Array,
):
    del B_x
    xt = jnp.swapaxes(A_x, 1, 2)
    w2t = B_w2.T
    hbm = pl.BlockSpec(memory_space=pl.ANY)
    slabs = pltpu.VMEM((NB, D, L), jnp.float32)
    out_t = pl.pallas_call(
        _kernel,
        grid=(1,),
        in_specs=[hbm] * 7,
        out_specs=hbm,
        out_shape=jax.ShapeDtypeStruct(xt.shape, xt.dtype),
        scratch_shapes=[
            pltpu.VMEM((D, S), jnp.bfloat16),
            pltpu.VMEM((D, S), jnp.bfloat16),
            pltpu.VMEM((D, S), jnp.bfloat16),
            pltpu.VMEM((1, D), jnp.bfloat16),
            pltpu.VMEM((D, 6 * D), jnp.bfloat16),
            pltpu.VMEM((D, 3 * D), jnp.bfloat16),
            pltpu.VMEM((D, D), jnp.bfloat16),
            pltpu.VMEM((D, DFF), jnp.bfloat16),
            pltpu.VMEM((D, DFF), jnp.bfloat16),
            pltpu.VMEM((6 * D, 128), jnp.float32),
            pltpu.VMEM((NCB, D, 128), jnp.float32),
            pltpu.VMEM((3 * D, D), jnp.bfloat16),
            pltpu.VMEM((D, D), jnp.bfloat16),
            pltpu.VMEM((DFF, D), jnp.bfloat16),
            pltpu.VMEM((NCB, S, 128), jnp.float32),
            pltpu.VMEM((D, S), jnp.float32),
            slabs, slabs, slabs, slabs, slabs,
            pltpu.VMEM((D, S), jnp.bfloat16),
            pltpu.SemaphoreType.DMA((16,)),
        ],
        compiler_params=pltpu.CompilerParams(
            dimension_semantics=("arbitrary",),
            vmem_limit_bytes=110 * 1024 * 1024,
        ),
    )(xt, c, w_mod, A_wqkv, A_wo, B_w1, w2t)
    return jnp.swapaxes(out_t, 1, 2)
```
